```python
import os as _os
_os.environ.setdefault("JAX_PLATFORMS", "cpu")
import jax
import jax.numpy as jnp

def _softmax(x, axis=-1):
    return jax.nn.softmax(x, axis=axis)
def _gelu(x):
    return jax.nn.gelu(x, approximate=True)
def _silu(x):
    return jax.nn.silu(x)
def _sigmoid(x):
    return jax.nn.sigmoid(x)
def _layernorm(x, axis=-1, eps=1e-5):
    m = jnp.mean(x, axis=axis, keepdims=True)
    v = jnp.var(x, axis=axis, keepdims=True)
    return (x - m) / jnp.sqrt(v + eps)
def _scatter_add(tgt, idx, src, axis=0):
    return tgt.at[idx].add(src)
def _segment_sum(src, seg, n):
    return jax.ops.segment_sum(src, seg, n)
class _Rng:
    def __init__(self, key):
        self._k = key
    def _next(self):
        self._k, sub = jax.random.split(self._k)
        return sub
    def normal(self, shape):
        return jax.random.normal(self._next(), shape, dtype=jnp.bfloat16)
    def randint(self, lo, hi, shape):
        return jax.random.randint(self._next(), shape, lo, hi, dtype=jnp.int32)
    def uniform(self, shape, lo=0.0, hi=1.0):
        return jax.random.uniform(self._next(), shape, jnp.bfloat16, lo, hi)
    def permutation(self, n):
        return jax.random.permutation(self._next(), n)


kernel_name = 'gated_mix__grouped_kv_mqa__ssm_conv_s5__prompt'

def setup_inputs():
    _rng = _Rng(jax.random.key(int.from_bytes(__import__("os").urandom(4), "little")))
    _w = (lambda a: (lambda t: t.astype(jnp.bfloat16) if jnp.issubdtype(t.dtype, jnp.floating) else t)(jnp.asarray(a)))
    def _A_setup():
        B, S, D, H = 1, 2048, 512, 32
        Dh = D // H
        return {
            "x": _w((lambda *s: _rng.normal(s) * 0.05)(B, S, D)),
            "wq": _w((lambda *s: _rng.normal(s) * 1.6)(D, H * Dh)),
            "wk": _w((lambda *s: _rng.normal(s) * 1.6)(D, Dh)),
            "wv": _w((lambda *s: _rng.normal(s) * 0.05)(D, Dh)),
            "wo": _w((lambda *s: _rng.normal(s) * 0.05)(H * Dh, D)),
        }
    _A_in = _A_setup()

    def _B_setup():
        B, S, D = 1, 2048, 512
        P = D
        Lambda_re = -0.5 * jnp.exp((lambda *s: _rng.normal(s) * 0.4)(P))
        Lambda_im = (lambda *s: _rng.normal(s) * 0.4)(P) * 1.0
        B_re = (lambda *s: _rng.normal(s) * 0.4)(P, D) * (D ** -0.5)
        B_im = (lambda *s: _rng.normal(s) * 0.4)(P, D) * (D ** -0.5)
        C_re = (lambda *s: _rng.normal(s) * 0.4)(D, P) * (P ** -0.5)
        C_im = (lambda *s: _rng.normal(s) * 0.4)(D, P) * (P ** -0.5)
        log_dt = (lambda *s: _rng.normal(s) * 0.4)(P) * 0.3 - 2.0
        Dskip = (lambda *s: _rng.normal(s) * 0.4)(D)
        return {
            "x": _w((lambda *s: _rng.normal(s) * 0.05)(B, S, D)),
            "Lambda_re": _w(Lambda_re),
            "Lambda_im": _w(Lambda_im),
            "B_re": _w(B_re),
            "B_im": _w(B_im),
            "C_re": _w(C_re),
            "C_im": _w(C_im),
            "log_dt": _w(log_dt),
            "Dskip": _w(Dskip),
        }
    _B_in = _B_setup()

    return {
        "A_x": _A_in["x"],
        "A_wq": _A_in["wq"],
        "A_wk": _A_in["wk"],
        "A_wv": _A_in["wv"],
        "A_wo": _A_in["wo"],
        "B_x": _B_in["x"],
        "B_Lambda_re": _B_in["Lambda_re"],
        "B_Lambda_im": _B_in["Lambda_im"],
        "B_B_re": _B_in["B_re"],
        "B_B_im": _B_in["B_im"],
        "B_C_re": _B_in["C_re"],
        "B_C_im": _B_in["C_im"],
        "B_log_dt": _B_in["log_dt"],
        "B_Dskip": _B_in["Dskip"],
        "gate_w": _w((lambda *s: _rng.normal(s) * 0.05)(512) * 16.0),
    }

def reference(A_x, A_wq, A_wk, A_wv, A_wo, B_x, B_Lambda_re, B_Lambda_im, B_B_re, B_B_im, B_C_re, B_C_im, B_log_dt, B_Dskip, gate_w):
    def _A_ref(x, wq, wk, wv, wo):
        B, S, D = x.shape
        H = 32
        Dh = D // H
        q = (lambda x, *d: x.transpose(*d))((x @ wq).reshape(B, S, H, Dh), 0, 2, 1, 3)
        k = x @ wk
        v = x @ wv
        scores = jnp.einsum("bhqd,bkd->bhqk", q, k) * (Dh ** -0.5)
        p = _softmax(scores, axis=-1)
        o = jnp.einsum("bhqk,bkd->bhqd", p, v)
        return (lambda x, *d: x.transpose(*d))(o, 0, 2, 1, 3).reshape(B, S, H * Dh) @ wo

    def _B_ref(x, Lambda_re, Lambda_im, B_re, B_im, C_re, C_im, log_dt, Dskip):
        Bsz, L, H = x.shape
        Lam = Lambda_re + 1j * Lambda_im
        Bmat = B_re + 1j * B_im
        Cmat = C_re + 1j * C_im
        dt = jnp.exp(log_dt)
        Lam_bar = jnp.exp(dt * Lam)
        B_bar = ((Lam_bar - 1.0) / Lam)[:, None] * Bmat
        Bu = jnp.einsum("bld,pd->blp", x + 0j, B_bar)
        h = jnp.zeros_like(Bu[:, 0, :])
        hs = []
        for t in range(L):
            h = Lam_bar[None, :] * h + Bu[:, t, :]
            hs.append(h)
        hseq = jnp.stack(hs, 1)
        y = 2.0 * jnp.einsum("blp,dp->bld", hseq, Cmat).real + x * Dskip[None, None, :]
        return y

    x = A_x
    g = _sigmoid((x * gate_w).sum(-1, keepdims=True))
    a = _A_ref(x, A_wq, A_wk, A_wv, A_wo)
    b = _B_ref(x, B_Lambda_re, B_Lambda_im, B_B_re, B_B_im, B_C_re, B_C_im, B_log_dt, B_Dskip)
    return g * a + (1 - g) * b
```

```python
import functools
import math

import jax
import jax.numpy as jnp
from jax import lax
import jax.experimental.pallas as pl
import jax.experimental.pallas.tpu as pltpu

S = 2048
D = 512
H = 32
DH = 16
TQ = 128
NB = S // TQ
KC = 128
NCH = S // KC
NC = 4
NG = H // NC
GW = NC * TQ
LAG = 2
QSCALE = (DH ** -0.5) * math.log2(math.e)
L_LO = 2.0 ** -80
L_HI = 2.0 ** 120

F32 = jnp.float32
BF16 = jnp.bfloat16
U32 = jnp.uint32


def _pk(x):
    return pltpu.bitcast(x, U32)


def _upk(x):
    return pltpu.bitcast(x, BF16)


def _nt(a, b):
    return lax.dot_general(a, b, (((1,), (1,)), ((), ())), preferred_element_type=F32)


def _cmul_add(ar, ai, sr, si, ur, ui):
    n = sr.shape[0] // 8
    sh = (n, 8, sr.shape[1])
    sr3, si3 = sr.reshape(sh), si.reshape(sh)
    re = (ar[None] * sr3 - ai[None] * si3).reshape(sr.shape) + ur
    im = (ar[None] * si3 + ai[None] * sr3).reshape(sr.shape) + ui
    return re, im


def _kernel(x_ref, wq_ref, wk_ref, wv_ref, wo_ref, lre_ref, lim_ref, bre_ref, bim_ref,
            cre_ref, cim_ref, ldt_ref, dsk_ref, gw_ref,
            out_ref,
            a_s, qg_s, k_s, vt_s, gt_s, gb_s, cp_s, par_s, ot_s, bp_s, out_s, sem):
    def row8(ref):
        return jnp.broadcast_to(ref[...].astype(F32).reshape(1, D), (8, D))

    a_s[0:256, :] = _pk(wq_ref[...].T)
    a_s[256:264, :] = _pk(wk_ref[...])
    a_s[264:272, :] = _pk(wv_ref[...])
    gw = gw_ref[...].reshape(1, D)
    rid = lax.broadcasted_iota(jnp.int32, (16, D), 0)
    a_s[272:280, :] = _pk(jnp.where(rid == 0, jnp.broadcast_to(gw.astype(F32), (16, D)), 0.0).astype(BF16))

    lre, lim = row8(lre_ref), row8(lim_ref)
    dt = jnp.exp(row8(ldt_ref)).astype(BF16).astype(F32)
    mag = jnp.exp(dt * lre)
    a1r, a1i = mag * jnp.cos(dt * lim), mag * jnp.sin(dt * lim)
    den = lre * lre + lim * lim
    nr, ni = a1r - 1.0, a1i
    cr = (nr * lre + ni * lim) / den
    ci = (ni * lre - nr * lim) / den
    a2r, a2i = a1r * a1r - a1i * a1i, 2.0 * a1r * a1i
    a4r, a4i = a2r * a2r - a2i * a2i, 2.0 * a2r * a2i
    a8r, a8i = a4r * a4r - a4i * a4i, 2.0 * a4r * a4i
    for n, v in enumerate((a1r, a1i, a2r, a2i, a4r, a4i, a8r, a8i, row8(dsk_ref))):
        par_s[n] = v
    c_re = cre_ref[...].astype(F32).reshape(D // 8, 8, D)
    c_im = cim_ref[...].astype(F32).reshape(D // 8, 8, D)
    cp_s[:, 0:D] = _pk((2.0 * (c_re * cr[None] - c_im * ci[None])).reshape(D, D).astype(BF16))
    cp_s[:, D:2 * D] = _pk((-2.0 * (c_re * ci[None] + c_im * cr[None])).reshape(D, D).astype(BF16))

    def proj_block(b):
        r0 = pl.multiple_of(b * TQ, TQ)
        xb = x_ref[0, pl.ds(r0, TQ), :]
        r = _nt(_upk(a_s[...]), xb)
        q = (r[0:D] * QSCALE).astype(BF16)
        qp = _pk(q)
        for g in range(NG):
            for c in range(NC):
                h = g * NC + c
                qg_s[b * NG + g, :, c * TQ:(c + 1) * TQ] = qp[8 * h:8 * h + 8]
        vt_s[:, pl.ds(r0, TQ)] = _pk(r[D + DH:D + 2 * DH].astype(BF16))
        g_t = jax.nn.sigmoid(r[D + 2 * DH:D + 2 * DH + 8])
        gt_s[b] = jnp.broadcast_to(g_t[0:1], (8, TQ))
        t = jnp.concatenate([r[D:D + DH], g_t, jnp.zeros((TQ - DH - 8, TQ), F32)], axis=0).T
        k_s[pl.ds(pl.multiple_of(b * (TQ // 2), TQ // 2), TQ // 2), :] = _pk(t[:, 0:DH].astype(BF16))
        gb_s[b] = 1.0 - jnp.broadcast_to(t[:, DH:DH + 1], (TQ, TQ))

    def proj_body(b, c):
        proj_block(b)
        return c
    lax.fori_loop(0, NB, proj_body, 0)

    vabs = jnp.abs(_upk(vt_s[...]).astype(F32))
    ot_s[0] = jnp.zeros(ot_s.shape[1:], U32)
    bp_s[0] = jnp.zeros(bp_s.shape[1:], F32)

    def final_block(slot_ot, slot_bp, slot_out):
        o = _upk(ot_s[slot_ot])
        o_t = jnp.concatenate([o[t * 128:(t + 1) * 128].T for t in range(D // 128)], axis=1)
        a = jnp.dot(o_t, wo_ref[...], preferred_element_type=F32)
        out_s[slot_out] = a + bp_s[slot_bp]

    def out_copy(blk):
        return pltpu.make_async_copy(out_s.at[blk], out_ref.at[0, pl.ds(blk * TQ, TQ)], sem)

    def ssm_u(i):
        xb = x_ref[0, pl.ds(pl.multiple_of(i * TQ, TQ), TQ), :]
        return xb, _nt(xb, bre_ref[...]), _nt(xb, bim_ref[...])

    def ssm_scan(ur, ui, carry):
        utr, uti, htr, hti = carry
        er = jnp.concatenate([utr, ur], axis=0)
        ei = jnp.concatenate([uti, ui], axis=0)
        for n, sh in ((0, 1), (2, 2), (4, 4)):
            er, ei = _cmul_add(par_s[n], par_s[n + 1], pltpu.roll(er, sh, 0), pltpu.roll(ei, sh, 0), er, ei)
        p8r, p8i = par_s[6], par_s[7]
        hr, hi = htr, hti
        outs_r, outs_i = [], []
        for r in range(TQ // 8):
            wr = er[8 + 8 * r:16 + 8 * r]
            wi = ei[8 + 8 * r:16 + 8 * r]
            hr, hi = p8r * hr - p8i * hi + wr, p8r * hi + p8i * hr + wi
            outs_r.append(hr)
            outs_i.append(hi)
        hcat = jnp.concatenate([jnp.concatenate(outs_r, axis=0), jnp.concatenate(outs_i, axis=0)], axis=1)
        return hcat.astype(BF16), (ur[TQ - 8:], ui[TQ - 8:], hr, hi)

    def ssm_y(i, xb, hb):
        y = _nt(hb, _upk(cp_s[...]))
        y = y + (xb.astype(F32).reshape(TQ // 8, 8, D) * par_s[8][None]).reshape(TQ, D)
        omg = gb_s[i]
        bp_s[i + 1] = y * jnp.concatenate([omg] * (D // TQ), axis=1)

    T = NG * NCH

    def body(i, carry):
        ssm_c, lmin, lmax = carry
        sc = {}
        ws = {}
        st = {}
        gt = gt_s[i]
        gt4 = jnp.concatenate([gt] * NC, axis=1)
        for t in range(T + LAG):
            if t == 0:
                final_block(i % 2, i, jnp.maximum(i - 1, 0))
            if t == 20:
                st["x"], st["ur"], st["ui"] = ssm_u(i)
            if t == 40:
                st["h"], ssm_c = ssm_scan(st["ur"], st["ui"], ssm_c)
            if t == 70:
                ssm_y(i, st["x"], st["h"])
            if t < T:
                g, j = divmod(t, NCH)
                if j == 0:
                    ws[g] = _upk(qg_s[i * NG + g])
                kk = _upk(k_s[j * (KC // 2):(j + 1) * (KC // 2), :])
                sc[t] = jnp.dot(kk, ws[g], preferred_element_type=F32)
            ts = t - LAG
            if ts < 0:
                continue
            g, j = divmod(ts, NCH)
            if j == 0:
                l8 = jnp.zeros((8, GW), F32)
                o = jnp.zeros((DH, GW), F32)
            p = jnp.exp2(sc.pop(ts))
            pr = p.reshape(KC // 8, 8, GW)
            for r in range(KC // 8):
                l8 = l8 + pr[r]
            vt = _upk(vt_s[:, j * KC:(j + 1) * KC])
            o = o + jnp.dot(vt, p.astype(BF16), preferred_element_type=F32)
            if j == NCH - 1:
                l = l8 + pltpu.roll(l8, 4, 0)
                l = l + pltpu.roll(l, 2, 0)
                l = l + pltpu.roll(l, 1, 0)
                for c in range(NC):
                    lc = l[:, c * TQ:(c + 1) * TQ]
                    lmin = jnp.minimum(lmin, lc)
                    lmax = jnp.maximum(lmax, lc)
                f = gt4 * pl.reciprocal(l, approx=False)
                on = (o.reshape(2, 8, GW) * f[None]).reshape(DH, GW).astype(BF16)
                onp = _pk(on)
                for c in range(NC):
                    hh = g * NC + c
                    ot_s[(i + 1) % 2, 8 * hh:8 * hh + 8, :] = onp[:, c * TQ:(c + 1) * TQ]

        @pl.when(i > 0)
        def _():
            out_copy(i - 1).start()
        return ssm_c, lmin, lmax

    z = jnp.zeros((8, D), F32)
    carry = ((z, z, z, z), jnp.full((8, TQ), jnp.inf, F32), jnp.zeros((8, TQ), F32))
    _, lmin, lmax = lax.fori_loop(0, NB, body, carry)
    final_block(NB % 2, NB, NB - 1)
    out_copy(NB - 1).start()
    for b in range(NB):
        out_copy(b).wait()

    vmax = jnp.max(vabs)
    ok = jnp.logical_and(lmin * jnp.minimum(vmax, 1.0) >= L_LO, lmax * jnp.maximum(vmax, 1.0) <= L_HI)
    unsafe = jnp.max(jnp.where(ok, 0.0, 1.0)) > 0.0

    @pl.when(unsafe)
    def _():
        FC = 256

        def blk_body(i, c0):
            gt = gt_s[i]
            gt4 = jnp.concatenate([gt] * NC, axis=1)

            def grp_body(g, c1):
                w = _upk(qg_s[i * NG + g])

                def scores(j):
                    kk = _upk(k_s[pl.ds(pl.multiple_of(j * (FC // 2), FC // 2), FC // 2), :])
                    return jnp.dot(kk, w, preferred_element_type=F32).reshape(FC // 8, 8, GW)

                def max_body(j, m8):
                    return jnp.maximum(m8, jnp.max(scores(j), axis=0))
                m = lax.fori_loop(0, S // FC, max_body, jnp.full((8, GW), -jnp.inf, F32))
                m = jnp.maximum(m, pltpu.roll(m, 4, 0))
                m = jnp.maximum(m, pltpu.roll(m, 2, 0))
                m = jnp.maximum(m, pltpu.roll(m, 1, 0))

                def sum_body(j, c2):
                    l8, o = c2
                    p = jnp.exp2(scores(j) - m[None])
                    vt = _upk(vt_s[:, pl.ds(pl.multiple_of(j * FC, FC), FC)])
                    o = o + jnp.dot(vt, p.reshape(FC, GW).astype(BF16), preferred_element_type=F32)
                    return l8 + jnp.sum(p, axis=0), o
                l8, o = lax.fori_loop(0, S // FC, sum_body,
                                      (jnp.zeros((8, GW), F32), jnp.zeros((DH, GW), F32)))
                l = l8 + pltpu.roll(l8, 4, 0)
                l = l + pltpu.roll(l, 2, 0)
                l = l + pltpu.roll(l, 1, 0)
                f = gt4 / l
                onp = _pk((o.reshape(2, 8, GW) * f[None]).reshape(DH, GW).astype(BF16))
                for c in range(NC):
                    ot_s[0, pl.ds(pl.multiple_of(8 * (g * NC + c), 8), 8), :] = onp[:, c * TQ:(c + 1) * TQ]
                return c1
            lax.fori_loop(0, NG, grp_body, 0)
            final_block(0, i + 1, i)
            cp = out_copy(i)
            cp.start()
            cp.wait()
            return c0
        lax.fori_loop(0, NB, blk_body, 0)


@jax.jit
def pallas_gated_mix__grouped_kv_mqa__ssm_conv_s5__prompt_kernel(
    A_x, A_wq, A_wk, A_wv, A_wo, B_x, B_Lambda_re, B_Lambda_im, B_B_re, B_B_im,
    B_C_re, B_C_im, B_log_dt, B_Dskip, gate_w,
):
    del B_x
    vm = pl.BlockSpec(memory_space=pltpu.VMEM)
    return pl.pallas_call(
        _kernel,
        out_shape=jax.ShapeDtypeStruct((1, S, D), F32),
        in_specs=[vm] * 14,
        out_specs=pl.BlockSpec(memory_space=pl.ANY),
        scratch_shapes=[
            pltpu.VMEM((280, D), U32),
            pltpu.VMEM((NB * NG, 8, GW), U32),
            pltpu.VMEM((S // 2, DH), U32),
            pltpu.VMEM((8, S), U32),
            pltpu.VMEM((NB, 8, TQ), F32),
            pltpu.VMEM((NB, TQ, TQ), F32),
            pltpu.VMEM((D // 2, 2 * D), U32),
            pltpu.VMEM((9, 8, D), F32),
            pltpu.VMEM((2, D // 2, TQ), U32),
            pltpu.VMEM((NB + 1, TQ, D), F32),
            pltpu.VMEM((NB, TQ, D), F32),
            pltpu.SemaphoreType.DMA(()),
        ],
        compiler_params=pltpu.CompilerParams(vmem_limit_bytes=64 * 2 ** 20),
    )(A_x, A_wq, A_wk.T, A_wv.T, A_wo, B_Lambda_re, B_Lambda_im, B_B_re, B_B_im,
      B_C_re, B_C_im, B_log_dt, B_Dskip, gate_w)
```

```python
import math

import jax
import jax.numpy as jnp
from jax import lax
import jax.experimental.pallas as pl
import jax.experimental.pallas.tpu as pltpu

S = 2048
D = 512
H = 32
DH = 16
TQ = 128
NB = S // TQ
KC = 128
NT = S // KC
NC = 4
NG = H // NC
GW = NC * TQ
NM = 7
SKEW = 3
KOPS = [SKEW] + [NM] * (NT - 1) + [NM - SKEW]
KO0 = [sum(KOPS[:n]) for n in range(len(KOPS) + 1)]
NKO = len(KOPS)
PV_AFTER = [v + 2 if v < NT - 2 else v + 3 for v in range(NT)]
T_U, T_SCAN, T_Y = 12, 14, 63
X0 = 4 * TQ
QSCALE = (DH ** -0.5) * math.log2(math.e)
L_LO = 2.0 ** -80
L_HI = 2.0 ** 120

F32 = jnp.float32
BF16 = jnp.bfloat16
U32 = jnp.uint32


def _pk(x):
    return pltpu.bitcast(x, U32)


def _upk(x):
    return pltpu.bitcast(x, BF16)


def _nn(a, b):
    return jnp.dot(a, b, preferred_element_type=F32)


def _nt(a, b):
    return lax.dot_general(a, b, (((1,), (1,)), ((), ())), preferred_element_type=F32)


def _rows(v, x):
    return (x.reshape(x.shape[0] // 8, 8, x.shape[1]) * v[None]).reshape(x.shape)


def _sum8(x):
    for sh in (4, 2, 1):
        x = x + pltpu.roll(x, sh, 0)
    return x


def _max8(x):
    for sh in (4, 2, 1):
        x = jnp.maximum(x, pltpu.roll(x, sh, 0))
    return x


def _kernel(x_h, wq_h, wk_h, wv_h, wo_h, lre_h, lim_h, bre_h, bim_h, cre_h, cim_h, ldt_h, dsk_h, gw_h,
            out_h,
            x_s, wq_s, wkv_s, wo_s, bre_s, bim_s, cre_s, cim_s, lre_s, lim_s, ldt_s, dsk_s, gw_s,
            a_s, qg_s, qf_s, kb_s, km_s, k_s, vt_s, gt_s, gb_s, par_s, u_s, ot_s, bp_s, out_s,
            zv_s, zs_s, isem, osem):
    cps = {}

    def fetch(name, src, dst):
        cps[name] = pltpu.make_async_copy(src, dst, isem.at[len(cps)])
        cps[name].start()

    def wait(*names):
        for n in names:
            cps[n].wait()

    fetch("wq", wq_h.bitcast(U32), wq_s)
    fetch("gw", gw_h, gw_s)
    fetch("wk", wk_h.bitcast(U32), wkv_s.at[0])
    fetch("wv", wv_h.bitcast(U32), wkv_s.at[1])
    fetch("x0", x_h.at[0, pl.ds(0, X0)].bitcast(U32), x_s.at[pl.ds(0, X0 // 2)])
    fetch("x1", x_h.at[0, pl.ds(X0, S - X0)].bitcast(U32), x_s.at[pl.ds(X0 // 2, (S - X0) // 2)])
    fetch("lre", lre_h, lre_s)
    fetch("lim", lim_h, lim_s)
    fetch("ldt", ldt_h, ldt_s)
    fetch("dsk", dsk_h, dsk_s)

    wait("gw", "wk", "wv", "wq")
    a_s[0:256, :] = _pk(_upk(wq_s[...]).T)
    a_s[256:264, :] = wkv_s[0]
    a_s[264:272, :] = wkv_s[1]
    rid = lax.broadcasted_iota(jnp.int32, (16, D), 0)
    gw = jnp.broadcast_to(gw_s[...].reshape(1, D).astype(F32), (16, D))
    a_s[272:280, :] = _pk(jnp.where(rid == 0, gw, 0.0).astype(BF16))

    def ssm_params():
        def row8(ref):
            return jnp.broadcast_to(ref[...].astype(F32).reshape(1, D), (8, D))
        lre, lim = row8(lre_s), row8(lim_s)
        dt = jnp.exp(row8(ldt_s)).astype(BF16).astype(F32)
        mag = jnp.exp(dt * lre)
        a1r, a1i = mag * jnp.cos(dt * lim), mag * jnp.sin(dt * lim)
        den = lre * lre + lim * lim
        cr = 2.0 * ((a1r - 1.0) * lre + a1i * lim) / den
        ci = 2.0 * (a1i * lre - (a1r - 1.0) * lim) / den
        a2r, a2i = a1r * a1r - a1i * a1i, 2.0 * a1r * a1i
        a4r, a4i = a2r * a2r - a2i * a2i, 2.0 * a2r * a2i
        a8r, a8i = a4r * a4r - a4i * a4i, 2.0 * a4r * a4i
        for n, v in enumerate((a1r, a1i, a2r, a2i, a4r, a4i, a8r, a8i, row8(dsk_s), cr, ci)):
            par_s[n] = v

    def proj_mm(b):
        return _nt(_upk(a_s[...]), _upk(x_s[b * (TQ // 2):(b + 1) * (TQ // 2), :]))

    def proj_post(b, r):
        q = (r[0:D] * QSCALE).astype(BF16)
        qp = _pk(q)
        for h in range(H):
            qg_s[b * NG + h // NC, :, (h % NC) * TQ:(h % NC + 1) * TQ] = qp[8 * h:8 * h + 8]
        qf_s[b] = q.astype(F32)
        vt_s[:, b * TQ:(b + 1) * TQ] = _pk(r[D + DH:D + 2 * DH].astype(BF16))
        g_t = jax.nn.sigmoid(r[D + 2 * DH:D + 2 * DH + 8])
        gt_s[b] = jnp.broadcast_to(g_t[0:1], (8, TQ))
        t = jnp.concatenate([r[D:D + DH], g_t, jnp.zeros((8, TQ), F32)], axis=0).T
        k16 = t[:, 0:DH].astype(BF16)
        kp = _pk(k16)
        k_s[b * (TQ // 2):(b + 1) * (TQ // 2), :] = kp
        for n in range(NM):
            km_s[8 * (b * NM + n):8 * (b * NM + n + 1), :] = kp[8 * (NM - n):8 * (NM - n + 1)]
        kf = k16.astype(F32)[0:16]
        for d in range(DH):
            kb_s[2 * b:2 * b + 2, d] = jnp.broadcast_to(kf[:, d:d + 1], (16, TQ)).reshape(2, 8, TQ)
        gb_s[b] = 1.0 - jnp.broadcast_to(t[:, DH:DH + 1], (TQ, TQ))

    wait("x0")
    r_prev = proj_mm(0)
    for b in range(1, NB + 1):
        if b == X0 // TQ:
            wait("x1")
            for name, src, dst in (("bre", bre_h, bre_s), ("bim", bim_h, bim_s), ("cre", cre_h, cre_s),
                                   ("cim", cim_h, cim_s), ("wo", wo_h, wo_s)):
                fetch(name, src.bitcast(U32), dst)
            wait("lre", "lim", "ldt", "dsk")
        r_next = proj_mm(b) if b < NB else None
        proj_post(b - 1, r_prev)
        r_prev = r_next
        if b == X0 // TQ + 1:
            ssm_params()

    vabs = jnp.abs(_upk(vt_s[...]).astype(F32))
    zv_s[...] = jnp.zeros(zv_s.shape, U32)
    zs_s[0] = 0
    ot_s[0] = jnp.zeros(ot_s.shape[1:], U32)
    bp_s[0] = jnp.zeros(bp_s.shape[1:], F32)
    wait("bre", "bim", "cre", "cim", "wo")

    def load_o(slot):
        o = _upk(ot_s[slot])
        return jnp.concatenate([o[t * 128:(t + 1) * 128].T for t in range(D // 128)], axis=1)

    def final_block(o, slot_bp, slot_out):
        out_s[slot_out] = _nn(o, _upk(wo_s[...])) + bp_s[slot_bp]

    def out_copy(blk):
        return pltpu.make_async_copy(out_s.at[blk], out_h.at[0, pl.ds(blk * TQ, TQ)], osem)

    def ssm_scan(carry):
        utr, uti, hr, hi = carry
        ur, ui = u_s[0, :, 0:D], u_s[0, :, D:2 * D]
        er = jnp.concatenate([utr, ur], axis=0)
        ei = jnp.concatenate([uti, ui], axis=0)
        for n, sh in ((0, 1), (2, 2), (4, 4)):
            ar, ai = par_s[n], par_s[n + 1]
            sr, si = pltpu.roll(er, sh, 0), pltpu.roll(ei, sh, 0)
            er, ei = _rows(ar, sr) - _rows(ai, si) + er, _rows(ar, si) + _rows(ai, sr) + ei
        p8r, p8i, cr, ci = par_s[6], par_s[7], par_s[9], par_s[10]
        yr, yi = [], []
        for r in range(1, TQ // 8 + 1):
            hr, hi = (p8r * hr - p8i * hi + er[8 * r:8 * r + 8], p8r * hi + p8i * hr + ei[8 * r:8 * r + 8])
            yr.append(cr * hr - ci * hi)
            yi.append(-(cr * hi + ci * hr))
        return (jnp.concatenate(yr, axis=0).astype(BF16), jnp.concatenate(yi, axis=0).astype(BF16),
                (ur[TQ - 8:], ui[TQ - 8:], hr, hi))

    def heads(x):
        return [x[:, c * TQ:(c + 1) * TQ] for c in range(NC)]

    T = NG * NKO

    def body(i, carry):
        ssm_c, lmin, lmax = carry
        zero = jnp.concatenate([zv_s[...]] * NC, axis=1)
        zs = zs_s[0]
        ws, qbs, pm = {}, {}, {}
        nxt = 0
        for t in range(T + 2):
            if t < T:
                g, j = divmod(t, NKO)
                if j == 0:
                    ws[g] = _upk(qg_s[i * NG + g])
                    qv = qf_s[i, g * NC * DH:(g + 1) * NC * DH, :]
                    qbs[g] = [[jnp.broadcast_to(qv[c * DH + d:c * DH + d + 1, :], (8, TQ))
                               for d in range(DH)] for c in range(NC)]
                p = jnp.exp2(_nn(_upk(km_s[8 * KO0[j]:8 * KO0[j + 1], :]), ws[g]))
                for n in range(KOPS[j]):
                    pm[(g, KO0[j] + n)] = p[16 * n:16 * n + 16]
            if t == 0:
                o_prev = load_o(i % 2)
            if t == T_U:
                xb = _upk(x_s[pl.ds(pl.multiple_of(i * (TQ // 2), TQ // 2), TQ // 2), :])
                u_s[0, :, 0:D] = _nt(xb, _upk(bre_s[...]))
                u_s[0, :, D:2 * D] = _nt(xb, _upk(bim_s[...]))
                u_s[zs + 1, 0:8, 0:TQ] = jnp.zeros((8, TQ), F32)
            if t == T_SCAN:
                hbr, hbi, ssm_c = ssm_scan(ssm_c)
            if t == T_Y:
                y = _nt(hbr, _upk(cre_s[...])) + _nt(hbi, _upk(cim_s[...])) + _rows(par_s[8], xb.astype(F32))
                bp_s[i + 1] = y * jnp.concatenate([gb_s[i]] * (D // TQ), axis=1)
            if t == T - 1:
                final_block(o_prev, i, jnp.maximum(i - 1, 0))
            g, j = divmod(nxt, NT)
            if nxt == NG * NT or g * NKO + PV_AFTER[j] != t:
                continue
            nxt += 1
            if nxt == 1:
                l8 = jnp.zeros((8, GW), F32)
                o = jnp.zeros((DH, GW), F32)
            elif j == 0:
                l8 = pltpu.bitcast(pltpu.bitcast(l8, U32) & zero, F32)
                o = pltpu.bitcast(pltpu.bitcast(o, U32) & jnp.concatenate([zero, zero], axis=0), F32)
            l = heads(l8)
            pv = [None] * NC
            blocks = []
            for n in range(NM):
                if n % 2 == 0:
                    c = n // 2
                    acc = [None, None]
                    for d in range(DH):
                        for k in range(2):
                            tt = kb_s[2 * j + k, d] * qbs[g][c][d]
                            acc[k] = tt if d == 0 else acc[k] + tt
                    pv[c] = [jnp.exp2(a) for a in acc]
                    l[c] = l[c] + pv[c][0] + pv[c][1]
                pb = pm.pop((g, NM * j + n))
                blocks.insert(0, pb)
                for r in range(2):
                    for c in range(NC):
                        l[c] = l[c] + pb[8 * r:8 * r + 8, c * TQ:(c + 1) * TQ]
            l8 = jnp.concatenate(l, axis=1)
            blocks.insert(0, jnp.concatenate([jnp.concatenate(x, axis=0) for x in pv], axis=1))
            o = o + _nn(_upk(vt_s[:, j * KC:(j + 1) * KC]), jnp.concatenate(blocks, axis=0).astype(BF16))
            if j == NT - 1:
                ls = _sum8(l8)
                for lc in heads(ls):
                    lmin = jnp.minimum(lmin, lc)
                    lmax = jnp.maximum(lmax, lc)
                f = jnp.concatenate([gt_s[i]] * NC, axis=1) * pltpu.reciprocal(ls, approx=False)
                onp = _pk(_rows(f, o).astype(BF16))
                for c in range(NC):
                    hh = g * NC + c
                    ot_s[(i + 1) % 2, 8 * hh:8 * hh + 8, :] = onp[:, c * TQ:(c + 1) * TQ]
        assert not pm and nxt == NG * NT

        @pl.when(i > 0)
        def _():
            out_copy(i - 1).start()
        return ssm_c, lmin, lmax

    z = jnp.zeros((8, D), F32)
    _, lmin, lmax = lax.fori_loop(
        0, NB, body, ((z, z, z, z), jnp.full((8, TQ), jnp.inf, F32), jnp.zeros((8, TQ), F32)))
    final_block(load_o(NB % 2), NB, NB - 1)
    out_copy(NB - 1).start()

    vmax = jnp.max(vabs)
    ok = jnp.logical_and(lmin * jnp.minimum(vmax, 1.0) >= L_LO, lmax * jnp.maximum(vmax, 1.0) <= L_HI)
    unsafe = jnp.max(jnp.where(ok, 0.0, 1.0)) > 0.0
    for b in range(NB):
        out_copy(b).wait()

    @pl.when(unsafe)
    def _():
        FC = 512

        def blk_body(i, c0):
            def grp_body(g, c1):
                w = _upk(qg_s[i * NG + g])

                def scores(j):
                    return _nn(_upk(k_s[j * (FC // 2):(j + 1) * (FC // 2), :]), w).reshape(FC // 8, 8, GW)

                m = jnp.max(scores(0), axis=0)
                for j in range(1, S // FC):
                    m = jnp.maximum(m, jnp.max(scores(j), axis=0))
                m = _max8(m)
                l8 = jnp.zeros((8, GW), F32)
                o = jnp.zeros((DH, GW), F32)
                for j in range(S // FC):
                    p = jnp.exp2(scores(j) - m[None])
                    l8 = l8 + jnp.sum(p, axis=0)
                    o = o + _nn(_upk(vt_s[:, j * FC:(j + 1) * FC]), p.reshape(FC, GW).astype(BF16))
                onp = _pk(_rows(jnp.concatenate([gt_s[i]] * NC, axis=1) / _sum8(l8), o).astype(BF16))
                for c in range(NC):
                    ot_s[0, pl.ds(pl.multiple_of(8 * (g * NC + c), 8), 8), :] = onp[:, c * TQ:(c + 1) * TQ]
                return c1
            lax.fori_loop(0, NG, grp_body, 0)
            final_block(load_o(0), i + 1, i)
            cp = out_copy(i)
            cp.start()
            cp.wait()
            return c0
        lax.fori_loop(0, NB, blk_body, 0)


@jax.jit
def pallas_gated_mix__grouped_kv_mqa__ssm_conv_s5__prompt_kernel(
    A_x: jax.Array,
    A_wq: jax.Array,
    A_wk: jax.Array,
    A_wv: jax.Array,
    A_wo: jax.Array,
    B_x: jax.Array,
    B_Lambda_re: jax.Array,
    B_Lambda_im: jax.Array,
    B_B_re: jax.Array,
    B_B_im: jax.Array,
    B_C_re: jax.Array,
    B_C_im: jax.Array,
    B_log_dt: jax.Array,
    B_Dskip: jax.Array,
    gate_w: jax.Array,
):
    del B_x
    hbm = pl.BlockSpec(memory_space=pl.ANY)
    mat = pltpu.VMEM((D // 2, D), U32)
    vec = pltpu.VMEM((D,), BF16)
    return pl.pallas_call(
        _kernel,
        out_shape=jax.ShapeDtypeStruct((1, S, D), F32),
        in_specs=[hbm] * 14,
        out_specs=hbm,
        scratch_shapes=[
            pltpu.VMEM((S // 2, D), U32),
            mat,
            pltpu.VMEM((2, DH // 2, D), U32),
            mat, mat, mat, mat, mat,
            vec, vec, vec, vec, vec,
            pltpu.VMEM((280, D), U32),
            pltpu.VMEM((NB * NG, 8, GW), U32),
            pltpu.VMEM((NB, D, TQ), F32),
            pltpu.VMEM((2 * NT, DH, 8, TQ), F32),
            pltpu.VMEM((8 * NM * NT, DH), U32),
            pltpu.VMEM((S // 2, DH), U32),
            pltpu.VMEM((8, S), U32),
            pltpu.VMEM((NB, 8, TQ), F32),
            pltpu.VMEM((NB, TQ, TQ), F32),
            pltpu.VMEM((11, 8, D), F32),
            pltpu.VMEM((2, TQ, 2 * D), F32),
            pltpu.VMEM((2, D // 2, TQ), U32),
            pltpu.VMEM((NB + 1, TQ, D), F32),
            pltpu.VMEM((NB, TQ, D), F32),
            pltpu.VMEM((8, TQ), U32),
            pltpu.SMEM((1,), jnp.int32),
            pltpu.SemaphoreType.DMA((15,)),
            pltpu.SemaphoreType.DMA(()),
        ],
        compiler_params=pltpu.CompilerParams(vmem_limit_bytes=64 * 2 ** 20),
    )(A_x, A_wq, A_wk.T, A_wv.T, A_wo, B_Lambda_re, B_Lambda_im, B_B_re, B_B_im,
      B_C_re, B_C_im, B_log_dt, B_Dskip, gate_w)
```

```python
import math

import jax
import jax.numpy as jnp
from jax import lax
import jax.experimental.pallas as pl
import jax.experimental.pallas.tpu as pltpu

S = 2048
D = 512
H = 32
DH = 16
TQ = 128
NB = S // TQ
KC = 128
NT = S // KC
NC = 4
NG = H // NC
GW = NC * TQ
NM = 7
SKEW = 3
KOPS = [SKEW] + [NM] * (NT - 1) + [NM - SKEW]
KO0 = [sum(KOPS[:n]) for n in range(len(KOPS) + 1)]
NKO = len(KOPS)
PV_AFTER = [v + 2 if v < NT - 2 else v + 3 for v in range(NT)]
T_U, T_SCAN, T_Y = 12, 14, 63
X0 = 4 * TQ
QSCALE = (DH ** -0.5) * math.log2(math.e)
L_LO = 2.0 ** -80
L_HI = 2.0 ** 120

F32 = jnp.float32
BF16 = jnp.bfloat16
U32 = jnp.uint32


def _pk(x):
    return pltpu.bitcast(x, U32)


def _upk(x):
    return pltpu.bitcast(x, BF16)


def _nn(a, b):
    return jnp.dot(a, b, preferred_element_type=F32)


def _nt(a, b):
    return lax.dot_general(a, b, (((1,), (1,)), ((), ())), preferred_element_type=F32)


def _rows(v, x):
    return (x.reshape(x.shape[0] // 8, 8, x.shape[1]) * v[None]).reshape(x.shape)


def _sum8(x):
    for sh in (4, 2, 1):
        x = x + pltpu.roll(x, sh, 0)
    return x


def _max8(x):
    for sh in (4, 2, 1):
        x = jnp.maximum(x, pltpu.roll(x, sh, 0))
    return x


def _kernel(x_h, wq_h, wk_h, wv_h, wo_h, lre_h, lim_h, bre_h, bim_h, cre_h, cim_h, ldt_h, dsk_h, gw_h,
            out_h,
            x_s, wq_s, wkv_s, wo_s, bre_s, bim_s, cre_s, cim_s, lre_s, lim_s, ldt_s, dsk_s, gw_s,
            a_s, qg_s, qf_s, kb_s, km_s, k_s, vt_s, gt_s, gb_s, par_s, u_s, ot_s, bp_s, out_s,
            zv_s, zs_s, isem, osem):
    cps = {}

    def fetch(name, src, dst):
        cps[name] = pltpu.make_async_copy(src, dst, isem.at[len(cps)])
        cps[name].start()

    def wait(*names):
        for n in names:
            cps[n].wait()

    fetch("wq", wq_h.bitcast(U32), wq_s)
    fetch("gw", gw_h, gw_s)
    fetch("wk", wk_h.bitcast(U32), wkv_s.at[0])
    fetch("wv", wv_h.bitcast(U32), wkv_s.at[1])
    fetch("x0", x_h.at[0, pl.ds(0, X0)].bitcast(U32), x_s.at[pl.ds(0, X0 // 2)])
    fetch("x1", x_h.at[0, pl.ds(X0, S - X0)].bitcast(U32), x_s.at[pl.ds(X0 // 2, (S - X0) // 2)])
    fetch("lre", lre_h, lre_s)
    fetch("lim", lim_h, lim_s)
    fetch("ldt", ldt_h, ldt_s)
    fetch("dsk", dsk_h, dsk_s)

    wait("gw", "wk", "wv", "wq")
    a_s[0:256, :] = _pk(_upk(wq_s[...]).T)
    a_s[256:264, :] = wkv_s[0]
    a_s[264:272, :] = wkv_s[1]
    rid = lax.broadcasted_iota(jnp.int32, (16, D), 0)
    gw = jnp.broadcast_to(gw_s[...].reshape(1, D).astype(F32), (16, D))
    a_s[272:280, :] = _pk(jnp.where(rid == 0, gw, 0.0).astype(BF16))

    def ssm_params():
        def row8(ref):
            return jnp.broadcast_to(ref[...].astype(F32).reshape(1, D), (8, D))
        lre, lim = row8(lre_s), row8(lim_s)
        dt = jnp.exp(row8(ldt_s)).astype(BF16).astype(F32)
        mag = jnp.exp(dt * lre)
        a1r, a1i = mag * jnp.cos(dt * lim), mag * jnp.sin(dt * lim)
        big = jnp.maximum(jnp.abs(lre), jnp.abs(lim))
        nre, nim = lre / big, lim / big
        den = nre * nre + nim * nim
        cr = 2.0 * ((a1r - 1.0) * nre + a1i * nim) / den / big
        ci = 2.0 * (a1i * nre - (a1r - 1.0) * nim) / den / big
        a2r, a2i = a1r * a1r - a1i * a1i, 2.0 * a1r * a1i
        a4r, a4i = a2r * a2r - a2i * a2i, 2.0 * a2r * a2i
        a8r, a8i = a4r * a4r - a4i * a4i, 2.0 * a4r * a4i
        for n, v in enumerate((a1r, a1i, a2r, a2i, a4r, a4i, a8r, a8i, row8(dsk_s), cr, ci)):
            par_s[n] = v

    def proj_mm(b):
        return _nt(_upk(a_s[...]), _upk(x_s[b * (TQ // 2):(b + 1) * (TQ // 2), :]))

    def proj_post(b, r):
        q = (r[0:D] * QSCALE).astype(BF16)
        qp = _pk(q)
        for h in range(H):
            qg_s[b * NG + h // NC, :, (h % NC) * TQ:(h % NC + 1) * TQ] = qp[8 * h:8 * h + 8]
        qf_s[b] = q.astype(F32)
        vt_s[:, b * TQ:(b + 1) * TQ] = _pk(r[D + DH:D + 2 * DH].astype(BF16))
        g_t = jax.nn.sigmoid(r[D + 2 * DH:D + 2 * DH + 8])
        gt_s[b] = jnp.broadcast_to(g_t[0:1], (8, TQ))
        t = jnp.concatenate([r[D:D + DH], g_t, jnp.zeros((8, TQ), F32)], axis=0).T
        k16 = t[:, 0:DH].astype(BF16)
        kp = _pk(k16)
        k_s[b * (TQ // 2):(b + 1) * (TQ // 2), :] = kp
        for n in range(NM):
            km_s[8 * (b * NM + n):8 * (b * NM + n + 1), :] = kp[8 * (NM - n):8 * (NM - n + 1)]
        kf = k16.astype(F32)[0:16]
        for d in range(DH):
            kb_s[2 * b:2 * b + 2, d] = jnp.broadcast_to(kf[:, d:d + 1], (16, TQ)).reshape(2, 8, TQ)
        gb_s[b] = 1.0 - jnp.broadcast_to(t[:, DH:DH + 1], (TQ, TQ))

    wait("x0")
    r_prev = proj_mm(0)
    for b in range(1, NB + 1):
        if b == X0 // TQ:
            wait("x1")
            for name, src, dst in (("bre", bre_h, bre_s), ("bim", bim_h, bim_s), ("cre", cre_h, cre_s),
                                   ("cim", cim_h, cim_s), ("wo", wo_h, wo_s)):
                fetch(name, src.bitcast(U32), dst)
            wait("lre", "lim", "ldt", "dsk")
        r_next = proj_mm(b) if b < NB else None
        proj_post(b - 1, r_prev)
        r_prev = r_next
        if b == X0 // TQ + 1:
            ssm_params()

    vabs = jnp.abs(_upk(vt_s[...]).astype(F32))
    zv_s[...] = jnp.zeros(zv_s.shape, U32)
    zs_s[0] = 0
    ot_s[0] = jnp.zeros(ot_s.shape[1:], U32)
    bp_s[0] = jnp.zeros(bp_s.shape[1:], F32)
    wait("bre", "bim", "cre", "cim", "wo")

    def load_o(slot):
        o = _upk(ot_s[slot])
        return jnp.concatenate([o[t * 128:(t + 1) * 128].T for t in range(D // 128)], axis=1)

    def final_block(o, slot_bp, slot_out):
        out_s[slot_out] = _nn(o, _upk(wo_s[...])) + bp_s[slot_bp]

    def out_copy(blk):
        return pltpu.make_async_copy(out_s.at[blk], out_h.at[0, pl.ds(blk * TQ, TQ)], osem)

    def ssm_scan(carry):
        utr, uti, hr, hi = carry
        ur, ui = u_s[0, :, 0:D], u_s[0, :, D:2 * D]
        er = jnp.concatenate([utr, ur], axis=0)
        ei = jnp.concatenate([uti, ui], axis=0)
        for n, sh in ((0, 1), (2, 2), (4, 4)):
            ar, ai = par_s[n], par_s[n + 1]
            sr, si = pltpu.roll(er, sh, 0), pltpu.roll(ei, sh, 0)
            er, ei = _rows(ar, sr) - _rows(ai, si) + er, _rows(ar, si) + _rows(ai, sr) + ei
        p8r, p8i, cr, ci = par_s[6], par_s[7], par_s[9], par_s[10]
        yr, yi = [], []
        for r in range(1, TQ // 8 + 1):
            hr, hi = (p8r * hr - p8i * hi + er[8 * r:8 * r + 8], p8r * hi + p8i * hr + ei[8 * r:8 * r + 8])
            yr.append(cr * hr - ci * hi)
            yi.append(-(cr * hi + ci * hr))
        return (jnp.concatenate(yr, axis=0).astype(BF16), jnp.concatenate(yi, axis=0).astype(BF16),
                (ur[TQ - 8:], ui[TQ - 8:], hr, hi))

    def heads(x):
        return [x[:, c * TQ:(c + 1) * TQ] for c in range(NC)]

    T = NG * NKO

    def body(i, carry):
        ssm_c, lmin, lmax = carry
        zero = jnp.concatenate([zv_s[...]] * NC, axis=1)
        zs = zs_s[0]
        ws, qbs, pm = {}, {}, {}
        nxt = 0
        for t in range(T + 2):
            if t < T:
                g, j = divmod(t, NKO)
                if j == 0:
                    ws[g] = _upk(qg_s[i * NG + g])
                    qv = qf_s[i, g * NC * DH:(g + 1) * NC * DH, :]
                    qbs[g] = [[jnp.broadcast_to(qv[c * DH + d:c * DH + d + 1, :], (8, TQ))
                               for d in range(DH)] for c in range(NC)]
                p = jnp.exp2(_nn(_upk(km_s[8 * KO0[j]:8 * KO0[j + 1], :]), ws[g]))
                for n in range(KOPS[j]):
                    pm[(g, KO0[j] + n)] = p[16 * n:16 * n + 16]
            if t == 0:
                o_prev = load_o(i % 2)
            if t == T_U:
                xb = _upk(x_s[pl.ds(pl.multiple_of(i * (TQ // 2), TQ // 2), TQ // 2), :])
                u_s[0, :, 0:D] = _nt(xb, _upk(bre_s[...]))
                u_s[0, :, D:2 * D] = _nt(xb, _upk(bim_s[...]))
                u_s[zs + 1, 0:8, 0:TQ] = jnp.zeros((8, TQ), F32)
            if t == T_SCAN:
                hbr, hbi, ssm_c = ssm_scan(ssm_c)
            if t == T_Y:
                y = _nt(hbr, _upk(cre_s[...])) + _nt(hbi, _upk(cim_s[...])) + _rows(par_s[8], xb.astype(F32))
                bp_s[i + 1] = y * jnp.concatenate([gb_s[i]] * (D // TQ), axis=1)
            if t == T - 1:
                final_block(o_prev, i, jnp.maximum(i - 1, 0))
            g, j = divmod(nxt, NT)
            if nxt == NG * NT or g * NKO + PV_AFTER[j] != t:
                continue
            nxt += 1
            if nxt == 1:
                l8 = jnp.zeros((8, GW), F32)
                o = jnp.zeros((DH, GW), F32)
            elif j == 0:
                l8 = pltpu.bitcast(pltpu.bitcast(l8, U32) & zero, F32)
                o = pltpu.bitcast(pltpu.bitcast(o, U32) & jnp.concatenate([zero, zero], axis=0), F32)
            l = heads(l8)
            pv = [None] * NC
            blocks = []
            for n in range(NM):
                if n % 2 == 0:
                    c = n // 2
                    acc = [None, None]
                    for d in range(DH):
                        for k in range(2):
                            tt = kb_s[2 * j + k, d] * qbs[g][c][d]
                            acc[k] = tt if d == 0 else acc[k] + tt
                    pv[c] = [jnp.exp2(a) for a in acc]
                    l[c] = l[c] + pv[c][0] + pv[c][1]
                pb = pm.pop((g, NM * j + n))
                blocks.insert(0, pb)
                for r in range(2):
                    for c in range(NC):
                        l[c] = l[c] + pb[8 * r:8 * r + 8, c * TQ:(c + 1) * TQ]
            l8 = jnp.concatenate(l, axis=1)
            blocks.insert(0, jnp.concatenate([jnp.concatenate(x, axis=0) for x in pv], axis=1))
            o = o + _nn(_upk(vt_s[:, j * KC:(j + 1) * KC]), jnp.concatenate(blocks, axis=0).astype(BF16))
            if j == NT - 1:
                ls = _sum8(l8)
                for lc in heads(ls):
                    lmin = jnp.minimum(lmin, lc)
                    lmax = jnp.maximum(lmax, lc)
                f = jnp.concatenate([gt_s[i]] * NC, axis=1) * pltpu.reciprocal(ls, approx=False)
                onp = _pk(_rows(f, o).astype(BF16))
                for c in range(NC):
                    hh = g * NC + c
                    ot_s[(i + 1) % 2, 8 * hh:8 * hh + 8, :] = onp[:, c * TQ:(c + 1) * TQ]
        assert not pm and nxt == NG * NT

        @pl.when(i > 0)
        def _():
            out_copy(i - 1).start()
        return ssm_c, lmin, lmax

    z = jnp.zeros((8, D), F32)
    _, lmin, lmax = lax.fori_loop(
        0, NB, body, ((z, z, z, z), jnp.full((8, TQ), jnp.inf, F32), jnp.zeros((8, TQ), F32)))
    final_block(load_o(NB % 2), NB, NB - 1)
    out_copy(NB - 1).start()

    vmax = jnp.max(vabs)
    ok = jnp.logical_and(lmin * jnp.minimum(vmax, 1.0) >= L_LO, lmax * jnp.maximum(vmax, 1.0) <= L_HI)
    unsafe = jnp.max(jnp.where(ok, 0.0, 1.0)) > 0.0
    for b in range(NB):
        out_copy(b).wait()

    @pl.when(unsafe)
    def _():
        FC = 512

        def blk_body(i, c0):
            def grp_body(g, c1):
                w = _upk(qg_s[i * NG + g])

                def scores(j):
                    return _nn(_upk(k_s[j * (FC // 2):(j + 1) * (FC // 2), :]), w).reshape(FC // 8, 8, GW)

                m = jnp.max(scores(0), axis=0)
                for j in range(1, S // FC):
                    m = jnp.maximum(m, jnp.max(scores(j), axis=0))
                m = _max8(m)
                l8 = jnp.zeros((8, GW), F32)
                o = jnp.zeros((DH, GW), F32)
                for j in range(S // FC):
                    p = jnp.exp2(scores(j) - m[None])
                    l8 = l8 + jnp.sum(p, axis=0)
                    o = o + _nn(_upk(vt_s[:, j * FC:(j + 1) * FC]), p.reshape(FC, GW).astype(BF16))
                onp = _pk(_rows(jnp.concatenate([gt_s[i]] * NC, axis=1) / _sum8(l8), o).astype(BF16))
                for c in range(NC):
                    ot_s[0, pl.ds(pl.multiple_of(8 * (g * NC + c), 8), 8), :] = onp[:, c * TQ:(c + 1) * TQ]
                return c1
            lax.fori_loop(0, NG, grp_body, 0)
            final_block(load_o(0), i + 1, i)
            cp = out_copy(i)
            cp.start()
            cp.wait()
            return c0
        lax.fori_loop(0, NB, blk_body, 0)


@jax.jit
def pallas_gated_mix__grouped_kv_mqa__ssm_conv_s5__prompt_kernel(
    A_x: jax.Array,
    A_wq: jax.Array,
    A_wk: jax.Array,
    A_wv: jax.Array,
    A_wo: jax.Array,
    B_x: jax.Array,
    B_Lambda_re: jax.Array,
    B_Lambda_im: jax.Array,
    B_B_re: jax.Array,
    B_B_im: jax.Array,
    B_C_re: jax.Array,
    B_C_im: jax.Array,
    B_log_dt: jax.Array,
    B_Dskip: jax.Array,
    gate_w: jax.Array,
):
    del B_x
    hbm = pl.BlockSpec(memory_space=pl.ANY)
    mat = pltpu.VMEM((D // 2, D), U32)
    vec = pltpu.VMEM((D,), BF16)
    return pl.pallas_call(
        _kernel,
        out_shape=jax.ShapeDtypeStruct((1, S, D), F32),
        in_specs=[hbm] * 14,
        out_specs=hbm,
        scratch_shapes=[
            pltpu.VMEM((S // 2, D), U32),
            mat,
            pltpu.VMEM((2, DH // 2, D), U32),
            mat, mat, mat, mat, mat,
            vec, vec, vec, vec, vec,
            pltpu.VMEM((280, D), U32),
            pltpu.VMEM((NB * NG, 8, GW), U32),
            pltpu.VMEM((NB, D, TQ), F32),
            pltpu.VMEM((2 * NT, DH, 8, TQ), F32),
            pltpu.VMEM((8 * NM * NT, DH), U32),
            pltpu.VMEM((S // 2, DH), U32),
            pltpu.VMEM((8, S), U32),
            pltpu.VMEM((NB, 8, TQ), F32),
            pltpu.VMEM((NB, TQ, TQ), F32),
            pltpu.VMEM((11, 8, D), F32),
            pltpu.VMEM((2, TQ, 2 * D), F32),
            pltpu.VMEM((2, D // 2, TQ), U32),
            pltpu.VMEM((NB + 1, TQ, D), F32),
            pltpu.VMEM((NB, TQ, D), F32),
            pltpu.VMEM((8, TQ), U32),
            pltpu.SMEM((1,), jnp.int32),
            pltpu.SemaphoreType.DMA((15,)),
            pltpu.SemaphoreType.DMA(()),
        ],
        compiler_params=pltpu.CompilerParams(vmem_limit_bytes=64 * 2 ** 20),
    )(A_x, A_wq, A_wk.T, A_wv.T, A_wo, B_Lambda_re, B_Lambda_im, B_B_re, B_B_im,
      B_C_re, B_C_im, B_log_dt, B_Dskip, gate_w)
```
